```python
import os as _os
_os.environ.setdefault("JAX_PLATFORMS", "cpu")
import jax
import jax.numpy as jnp

def _softmax(x, axis=-1):
    return jax.nn.softmax(x, axis=axis)
def _gelu(x):
    return jax.nn.gelu(x, approximate=True)
def _silu(x):
    return jax.nn.silu(x)
def _sigmoid(x):
    return jax.nn.sigmoid(x)
def _layernorm(x, axis=-1, eps=1e-5):
    m = jnp.mean(x, axis=axis, keepdims=True)
    v = jnp.var(x, axis=axis, keepdims=True)
    return (x - m) / jnp.sqrt(v + eps)
def _scatter_add(tgt, idx, src, axis=0):
    return tgt.at[idx].add(src)
def _segment_sum(src, seg, n):
    return jax.ops.segment_sum(src, seg, n)
class _Rng:
    def __init__(self, key):
        self._k = key
    def _next(self):
        self._k, sub = jax.random.split(self._k)
        return sub
    def normal(self, shape):
        return jax.random.normal(self._next(), shape, dtype=jnp.bfloat16)
    def randint(self, lo, hi, shape):
        return jax.random.randint(self._next(), shape, lo, hi, dtype=jnp.int32)
    def uniform(self, shape, lo=0.0, hi=1.0):
        return jax.random.uniform(self._next(), shape, jnp.bfloat16, lo, hi)
    def permutation(self, n):
        return jax.random.permutation(self._next(), n)


kernel_name = 'interleave_layers__gqa_block_cached__dense_activation_mish__decode'

def setup_inputs():
    _rng = _Rng(jax.random.key(int.from_bytes(__import__("os").urandom(4), "little")))
    _w = (lambda a: (lambda t: t.astype(jnp.bfloat16) if jnp.issubdtype(t.dtype, jnp.floating) else t)(jnp.asarray(a)))
    def _A_setup():
        B, Sq, D = 1, 1, 512
        Hq, Hkv, Sk, Dh = 32, 8, 65536, 128
        assert Hq % Hkv == 0, (Hq, Hkv)
        return {
            "x": _w((lambda *s: _rng.normal(s) * 0.05)(B, Sq, D)),
            "k_cache": _w((lambda *s: _rng.normal(s) * 1.6)(B, Hkv, Sk, Dh)),
            "v_cache": _w((lambda *s: _rng.normal(s) * 1.6)(B, Hkv, Sk, Dh)),
            "wq": _w((lambda *s: _rng.normal(s) * 1.6)(D, Hq * Dh) * (D ** -0.5)),
            "wo": _w((lambda *s: _rng.normal(s) * 1.6)(Hq * Dh, D) * ((Hq * Dh) ** -0.5)),
        }
    _A_in = _A_setup()

    def _B_setup():
        B, S, D, F = 1, 1, 512, 1792
        return {
            "x": _w((lambda *s: _rng.normal(s) * 0.05)(B, S, D)),
            "w1": _w((lambda *s: _rng.normal(s) * 0.8)(D, F) * (D ** -0.5)),
            "b1": _w((lambda *s: _rng.normal(s) * 0.8)(F)),
            "w2": _w((lambda *s: _rng.normal(s) * 0.8)(F, D) * (F ** -0.5)),
        }
    _B_in = _B_setup()

    return {
        "A_x": _A_in["x"],
        "A_k_cache": _A_in["k_cache"],
        "A_v_cache": _A_in["v_cache"],
        "A_wq": _A_in["wq"],
        "A_wo": _A_in["wo"],
        "B_x": _B_in["x"],
        "B_w1": _B_in["w1"],
        "B_b1": _B_in["b1"],
        "B_w2": _B_in["w2"],
    }

def reference(A_x, A_k_cache, A_v_cache, A_wq, A_wo, B_x, B_w1, B_b1, B_w2):
    def _A_ref(x, k_cache, v_cache, wq, wo):
        B, Sq, D = x.shape
        Hq, Dh = 32, 128
        Hkv = k_cache.shape[1]
        rep = Hq // Hkv
        q = (lambda x, *d: x.transpose(*d))((x @ wq).reshape(B, Sq, Hq, Dh), 0, 2, 1, 3)
        k = jnp.repeat(k_cache, rep, axis=1)
        v = jnp.repeat(v_cache, rep, axis=1)
        scores = jnp.einsum("bhqd,bhkd->bhqk", q, k) * (Dh ** -0.5)
        p = _softmax(scores, axis=-1)
        o = jnp.einsum("bhqk,bhkd->bhqd", p, v)
        return (lambda x, *d: x.transpose(*d))(o, 0, 2, 1, 3).reshape(B, Sq, Hq * Dh) @ wo

    def _B_ref(x, w1, b1, w2):
        h = jnp.einsum("bsd,df->bsf", x, w1) + b1
        sp = jnp.log1p(jnp.exp(-jnp.abs(h))) + jnp.where(h > 0, h, jnp.zeros_like(h))
        act = h * jnp.tanh(sp)
        return jnp.einsum("bsf,fd->bsd", act, w2)

    x = A_x
    x = x + _A_ref(_layernorm(x, axis=-1), A_k_cache, A_v_cache, A_wq, A_wo)
    x = x + _B_ref(_layernorm(x, axis=-1), B_w1, B_b1, B_w2)
    x = x + _A_ref(_layernorm(x, axis=-1), A_k_cache, A_v_cache, A_wq, A_wo)
    x = x + _B_ref(_layernorm(x, axis=-1), B_w1, B_b1, B_w2)
    return x
```

```python
import functools
import jax
import jax.numpy as jnp
from jax import lax
import jax.experimental.pallas as pl
import jax.experimental.pallas.tpu as pltpu

D = 512; F = 1792; HQ = 32; HKV = 8; SK = 65536; DH = 128; REP = 4
f32 = jnp.float32; bf16 = jnp.bfloat16
GW = REP * DH


def build(B=4096, S=4096, R=54, P=4, E=8, vmem_mb=128, skip_dma=False, skip_compute=False, b1mode="1d", SUB=128, pk=0, pv=1):
    T = HKV * SK // B
    CPH = SK // B
    NS = T - R
    NSLOT = R + P
    UB = R + NS - P
    scale = DH ** -0.5
    assert P <= CPH

    def rnd(x):
        return x.astype(bf16).astype(f32)

    def ln_bf16(x):
        mu = jnp.mean(x, axis=-1, keepdims=True)
        xc = x - mu
        var = jnp.mean(xc * xc, axis=-1, keepdims=True)
        return (xc / jnp.sqrt(var + 1e-5)).astype(bf16)

    def kernel(x_ref, b1_ref, k_hbm, v_hbm, wq_hbm, wo_hbm, w1_hbm, w2_hbm, o_ref,
               kbuf, vbuf, wq_v, wo_v, w1_v, w2_v, q_scr, m_scr, l_scr, acc_scr, at_scr, cnt,
               ksem, vsem, wsem):
        def k_copy(chunk, slot):
            return pltpu.make_async_copy(k_hbm.at[chunk], kbuf.at[slot], ksem.at[slot])

        def v_copy(chunk, slot):
            return pltpu.make_async_copy(v_hbm.at[chunk], vbuf.at[slot], vsem.at[slot])

        def start_kv(chunk, slot):
            if skip_dma: return
            for o in range(0, B, SUB):
                sl = pl.ds(o, min(SUB, B - o))
                pltpu.make_async_copy(k_hbm.at[chunk, sl], kbuf.at[slot, sl], ksem.at[slot]).start(priority=pk)
                pltpu.make_async_copy(v_hbm.at[chunk, sl], vbuf.at[slot, sl], vsem.at[slot]).start(priority=pv)

        wcopies = [pltpu.make_async_copy(wq_hbm, wq_v, wsem.at[0]),
                   pltpu.make_async_copy(wo_hbm, wo_v, wsem.at[1]),
                   pltpu.make_async_copy(w1_hbm, w1_v, wsem.at[2]),
                   pltpu.make_async_copy(w2_hbm, w2_v, wsem.at[3])]

        def slot1(c):
            if isinstance(c, int):
                return c if c < R else R + (c - R) % P
            return jnp.where(c < R, c, R + (c - R) % P)

        wcopies[0].start()
        for c in range(P):
            start_kv(c, slot1(c))
        for c in wcopies[1:]:
            c.start()

        row = lax.broadcasted_iota(jnp.int32, (8, DH), 0)

        def qproj(xn, heads):
            lo, hi = heads[0], heads[-1] + 1
            q8 = jnp.dot(xn, wq_v[:, lo * GW:hi * GW], preferred_element_type=f32)
            for g in heads:
                qg = jnp.zeros((8, DH), f32)
                for r in range(REP):
                    j = REP * (g - lo) + r
                    qg = jnp.where(row == r, q8[:, j * DH:(j + 1) * DH], qg)
                q_scr[g] = qg

        def init_state():
            m_scr[...] = jnp.full(m_scr.shape, -jnp.inf, f32)
            l_scr[...] = jnp.zeros(l_scr.shape, f32)
            acc_scr[...] = jnp.zeros(acc_scr.shape, f32)
            at_scr[...] = jnp.zeros(at_scr.shape, f32)
            for g in range(HKV):
                cnt[g] = 0

        def compute(slot, head, wait_k, wait_v):
            q = q_scr[head].astype(bf16)
            m = m_scr[head]
            l = l_scr[head]
            acc = acc_scr[head]
            for j in range(B // S):
                if j == 0:
                    wait_k()
                k = kbuf[slot, pl.ds(j * S, S), :]
                s = lax.dot_general(q, k, (((1,), (1,)), ((), ())), preferred_element_type=f32)
                m_cur = jnp.max(s, axis=1, keepdims=True)
                m_new = jnp.maximum(m, m_cur)
                alpha = jnp.exp((m - m_new) * scale)
                ps = [jnp.exp((s[:, t * 128:(t + 1) * 128] - m_new) * scale) for t in range(S // 128)]
                lsum = ps[0]
                for t in range(1, S // 128):
                    lsum = lsum + ps[t]
                l = l * alpha + lsum
                p = jnp.concatenate(ps, axis=1).astype(bf16)
                if j == 0:
                    wait_v()
                v = vbuf[slot, pl.ds(j * S, S), :]
                pv = jnp.dot(p, v, preferred_element_type=f32)
                acc = acc * alpha + pv
                m = m_new
            m_scr[head] = m
            l_scr[head] = l
            acc_scr[head] = acc

        def finalize(head):
            lt = jnp.sum(l_scr[head], axis=1, keepdims=True)
            og = acc_scr[head] / lt
            a = jnp.concatenate([jnp.where(row == r, og, 0.0).astype(bf16) for r in range(REP)], axis=1)
            w = wo_v[pl.ds(pl.multiple_of(head * GW, GW), GW), :]
            at_scr[...] += jnp.dot(a, w, preferred_element_type=f32)

        def visit(slot, chunk, wait_pred, first_pass):
            head = chunk // CPH

            def mkwait(cp):
                def w():
                    if skip_dma or wait_pred is False:
                        return
                    if wait_pred is None:
                        cp(0, slot).wait()
                    else:
                        @pl.when(wait_pred)
                        def _():
                            cp(0, slot).wait()
                return w
            if skip_compute:
                mkwait(k_copy)(); mkwait(v_copy)()
            else:
                compute(slot, head, mkwait(k_copy), mkwait(v_copy))
            return head

        def post(head, first_pass):
            n = cnt[head] + 1
            cnt[head] = n

            @pl.when(n == CPH)
            def _():
                if first_pass:
                    @pl.when(head == 0)
                    def _():
                        for c in wcopies[1:]:
                            c.wait()
                finalize(head)

        def pass1():
            def body(c, carry):
                head = visit(slot1(c), c, None, True)

                @pl.when(c + P < T)
                def _():
                    start_kv(c + P, slot1(c + P))
                post(head, True)
                return carry
            lax.fori_loop(0, T, body, 0)

        def pass2a():
            def body(i, carry):
                slot = R + (NS - P + i) % P
                head = visit(slot, T - P + i, False, False)
                start_kv(R + i, slot)
                post(head, False)
                return carry
            lax.fori_loop(0, P, body, 0)

        def pass2b():
            def rbf(u):
                return jnp.minimum(R, (u * R) // (UB - E))

            def body(u, carry):
                rb = rbf(u)
                is_res = rbf(u + 1) > rb
                s = u - rb
                slot = jnp.where(is_res, rb, R + (NS + s) % P)
                chunk = jnp.where(is_res, rb, R + s)
                head = visit(slot, chunk, jnp.logical_not(is_res), False)

                @pl.when(jnp.logical_and(jnp.logical_not(is_res), s + P < NS - P))
                def _():
                    start_kv(R + s + P, slot)
                post(head, False)
                return carry
            lax.fori_loop(0, UB, body, 0)

        def attn_out(x):
            at = jnp.sum(at_scr[...], axis=0, keepdims=True)
            return rnd(x + rnd(at))

        if b1mode == "1d":
            b1 = b1_ref[...].astype(f32).reshape(1, F)
        else:
            b1 = b1_ref[...].astype(f32)

        def mlp(x):
            xn = ln_bf16(x)
            h = rnd(rnd(jnp.dot(xn, w1_v[...], preferred_element_type=f32)) + b1)
            sp = jnp.log1p(jnp.exp(-jnp.abs(h))) + jnp.maximum(h, 0.0)
            act = (h * jnp.tanh(sp)).astype(bf16)
            y = jnp.dot(act, w2_v[...], preferred_element_type=f32)
            return rnd(x + rnd(y))

        x = jnp.broadcast_to(x_ref[...].astype(f32), (8, D))
        init_state()
        xn = ln_bf16(x)
        wcopies[0].wait()
        qproj(xn, list(range(HKV)))
        pass1()
        x = mlp(attn_out(x))
        xn = ln_bf16(x)
        qproj(xn, [HKV - 1])
        init_state()
        pass2a()
        qproj(xn, list(range(HKV - 1)))
        pass2b()
        x = mlp(attn_out(x))
        o_ref[...] = x[0:1, :].astype(o_ref.dtype)

    @jax.jit
    def fn(A_x, A_k_cache, A_v_cache, A_wq, A_wo, B_x, B_w1, B_b1, B_w2):
        x = A_x.reshape(1, D)
        k = A_k_cache.reshape(T, B, DH)
        v = A_v_cache.reshape(T, B, DH)
        b1 = B_b1 if b1mode == "1d" else B_b1.reshape(1, F)
        vm = pl.BlockSpec(memory_space=pltpu.VMEM)
        hb = pl.BlockSpec(memory_space=pl.ANY)
        out = pl.pallas_call(
            kernel,
            out_shape=jax.ShapeDtypeStruct((1, D), bf16),
            in_specs=[vm, vm, hb, hb, hb, hb, hb, hb],
            out_specs=vm,
            scratch_shapes=[
                pltpu.VMEM((NSLOT, B, DH), bf16),
                pltpu.VMEM((NSLOT, B, DH), bf16),
                pltpu.VMEM((D, HQ * DH), bf16),
                pltpu.VMEM((HQ * DH, D), bf16),
                pltpu.VMEM((D, F), bf16),
                pltpu.VMEM((F, D), bf16),
                pltpu.VMEM((HKV, 8, DH), f32),
                pltpu.VMEM((HKV, 8, DH), f32),
                pltpu.VMEM((HKV, 8, DH), f32),
                pltpu.VMEM((HKV, 8, DH), f32),
                pltpu.VMEM((8, D), f32),
                pltpu.SMEM((HKV,), jnp.int32),
                pltpu.SemaphoreType.DMA((NSLOT,)),
                pltpu.SemaphoreType.DMA((NSLOT,)),
                pltpu.SemaphoreType.DMA((4,)),
            ],
            compiler_params=pltpu.CompilerParams(vmem_limit_bytes=vmem_mb * 1024 * 1024),
        )(x, b1, k, v, A_wq, A_wo, B_w1, B_w2)
        return out.reshape(1, 1, D)
    return fn


_fn = build(**OPQ)


@jax.jit
def pallas_interleave_layers__gqa_block_cached__dense_activation_mish__decode_kernel(A_x, A_k_cache, A_v_cache, A_wq, A_wo, B_x, B_w1, B_b1, B_w2):
    return _fn(A_x, A_k_cache, A_v_cache, A_wq, A_wo, B_x, B_w1, B_b1, B_w2)
```

```python
import functools

import jax
import jax.numpy as jnp
from jax import lax
import jax.experimental.pallas as pl
import jax.experimental.pallas.tpu as pltpu

D = 512
F = 1792
HQ, HKV, SK, DH = 32, 8, 65536, 128
REP = HQ // HKV
GW = REP * DH

B = 4096
T = HKV * SK // B
CPH = SK // B
R = 54
P = 4
NS = T - R
NSLOT = R + P
E = 8
UB = R + NS - P
SUB = 160
HALF = B // 2
PIECES = [(s * HALF + o, min(SUB, HALF - o)) for o in range(0, HALF, SUB) for s in range(2)]
SCALE = DH ** -0.5

f32 = jnp.float32
bf16 = jnp.bfloat16


def _rnd(x):
    return x.astype(bf16).astype(f32)


def _ln_bf16(x):
    mu = jnp.mean(x, axis=-1, keepdims=True)
    xc = x - mu
    var = jnp.mean(xc * xc, axis=-1, keepdims=True)
    return (xc / jnp.sqrt(var + 1e-5)).astype(bf16)


def _kernel(x_ref, b1_ref, k_hbm, v_hbm, wq_hbm, wo_hbm, w1_hbm, w2_hbm, o_ref,
            kbuf, vbuf, wq_v, wo_v, w1_v, w2_v, q_scr, m_scr, l_scr, acc_scr, at_scr, cnt,
            ksem, vsem, wsem):

    def start_both(chunk, slot):
        for o, z in PIECES:
            sl = pl.ds(o, z)
            pltpu.make_async_copy(k_hbm.at[chunk, sl], kbuf.at[slot, sl], ksem.at[slot]).start(priority=0)
            pltpu.make_async_copy(v_hbm.at[chunk, sl], vbuf.at[slot, sl], vsem.at[slot]).start(priority=1)

    def start_one(src, buf, sem, chunk, slot):
        for n, (o, z) in enumerate(PIECES):
            sl = pl.ds(o, z)
            pltpu.make_async_copy(src.at[chunk, sl], buf.at[slot, sl], sem.at[slot]).start(priority=n % 2)

    def wait_one(buf, sem, slot):
        pltpu.make_async_copy(buf.at[slot], buf.at[slot], sem.at[slot]).wait()

    def wpieces(src_ref, dst_ref, sem, rb, cbs, prio):
        nr = src_ref.shape[0]
        ops = []
        for r0 in range(0, nr, rb):
            c0 = 0
            for cz in cbs:
                ops.append((r0, min(rb, nr - r0), c0, cz))
                c0 += cz

        def go(op):
            r0, rz, c0, cz = op
            pltpu.make_async_copy(src_ref.at[pl.ds(r0, rz), pl.ds(c0, cz)],
                                  dst_ref.at[pl.ds(r0, rz), pl.ds(c0, cz)], sem).start(priority=prio)
        return [functools.partial(go, op) for op in ops]

    def zipstart(a, b):
        for i in range(max(len(a), len(b))):
            if i < len(a):
                a[i]()
            if i < len(b):
                b[i]()

    def wwait(dst_ref, i):
        pltpu.make_async_copy(dst_ref, dst_ref, wsem.at[i]).wait()

    def slot1(c):
        if isinstance(c, int):
            return c if c < R else R + (c - R) % P
        return jnp.where(c < R, c, R + (c - R) % P)

    zipstart(wpieces(wq_hbm, wq_v, wsem.at[0], 16, [1408, 1408, 1280], 0),
             wpieces(wo_hbm, wo_v, wsem.at[1], 48, [D], 1))
    for c in range(P):
        start_both(c, slot1(c))
    zipstart(wpieces(w1_hbm, w1_v, wsem.at[2], 16, [F], 0),
             wpieces(w2_hbm, w2_v, wsem.at[3], 48, [D], 1))

    row = lax.broadcasted_iota(jnp.int32, (8, DH), 0)

    def qproj(xn, heads):
        lo, hi = heads[0], heads[-1] + 1
        q8 = jnp.dot(xn, wq_v[:, lo * GW:hi * GW], preferred_element_type=f32)
        for g in heads:
            qg = jnp.zeros((8, DH), f32)
            for r in range(REP):
                j = REP * (g - lo) + r
                qg = jnp.where(row == r, q8[:, j * DH:(j + 1) * DH], qg)
            q_scr[g] = qg

    def init_state():
        m_scr[...] = jnp.full(m_scr.shape, -jnp.inf, f32)
        l_scr[...] = jnp.zeros(l_scr.shape, f32)
        acc_scr[...] = jnp.zeros(acc_scr.shape, f32)
        at_scr[...] = jnp.zeros(at_scr.shape, f32)
        for g in range(HKV):
            cnt[g] = 0

    def attn_out(x):
        at = jnp.sum(at_scr[...], axis=0, keepdims=True)
        return _rnd(x + _rnd(at))

    b1 = b1_ref[...].astype(f32).reshape(1, F)

    def mlp(x):
        xn = _ln_bf16(x)
        h = _rnd(_rnd(jnp.dot(xn, w1_v[...], preferred_element_type=f32)) + b1)
        sp = jnp.log1p(jnp.exp(-jnp.abs(h))) + jnp.maximum(h, 0.0)
        act = (h * jnp.tanh(sp)).astype(bf16)
        y = jnp.dot(act, w2_v[...], preferred_element_type=f32)
        return _rnd(x + _rnd(y))

    def cond(pred, fn):
        if pred is True:
            fn()
        elif pred is not False:
            pl.when(pred)(fn)

    def visit(slot, chunk, do_wait, nchunk, nslot, do_issue, first_pass, early=False):
        head = chunk // CPH
        q = q_scr[head].astype(bf16)
        m = m_scr[head]
        cond(do_wait, lambda: wait_one(kbuf, ksem, slot))
        s = lax.dot_general(q, kbuf[slot], (((1,), (1,)), ((), ())), preferred_element_type=f32)
        if early:
            start_one(k_hbm, kbuf, ksem, nchunk, nslot)
        m_new = jnp.maximum(m, jnp.max(s, axis=1, keepdims=True))
        alpha = jnp.exp((m - m_new) * SCALE)
        ps = [jnp.exp((s[:, t * 128:(t + 1) * 128] - m_new) * SCALE) for t in range(B // 128)]
        lsum = ps[0]
        for t in range(1, B // 128):
            lsum = lsum + ps[t]
        p = jnp.concatenate(ps, axis=1).astype(bf16)
        cond(do_wait, lambda: wait_one(vbuf, vsem, slot))
        pv = jnp.dot(p, vbuf[slot], preferred_element_type=f32)
        m_scr[head] = m_new
        l_scr[head] = l_scr[head] * alpha + lsum
        acc_scr[head] = acc_scr[head] * alpha + pv
        if early:
            start_one(v_hbm, vbuf, vsem, nchunk, nslot)
        else:
            cond(do_issue, lambda: start_both(nchunk, nslot))

        n = cnt[head] + 1
        cnt[head] = n

        @pl.when(n == CPH)
        def _():
            if first_pass:
                @pl.when(head == 0)
                def _():
                    wwait(wo_v, 1)
                    wwait(w1_v, 2)
                    wwait(w2_v, 3)
            lt = jnp.sum(l_scr[head], axis=1, keepdims=True)
            og = acc_scr[head] / lt
            a = jnp.concatenate([jnp.where(row == r, og, 0.0).astype(bf16) for r in range(REP)], axis=1)
            w = wo_v[pl.ds(pl.multiple_of(head * GW, GW), GW), :]
            at_scr[...] += jnp.dot(a, w, preferred_element_type=f32)

    def pass1():
        def body(c, carry):
            nc = jnp.minimum(c + P, T - 1)
            visit(slot1(c), c, True, nc, slot1(nc), c + P < T, True)
            return carry
        lax.fori_loop(0, T, body, 0)

    def pass2a():
        def body(i, carry):
            slot = R + (NS - P + i) % P
            visit(slot, T - P + i, False, R + i, slot, True, False)
            return carry
        slot0 = R + (NS - P) % P
        visit(slot0, T - P, False, R, slot0, True, False, early=True)
        lax.fori_loop(1, P, body, 0)

    def pass2b():
        def rbf(u):
            return jnp.minimum(R, (u * R) // (UB - E))

        def body(u, carry):
            rb = rbf(u)
            is_res = rbf(u + 1) > rb
            strm = jnp.logical_not(is_res)
            s = u - rb
            slot = jnp.where(is_res, rb, R + (NS + s) % P)
            chunk = jnp.where(is_res, rb, R + s)
            nc = jnp.minimum(R + s + P, T - 1)
            visit(slot, chunk, strm, nc, slot, jnp.logical_and(strm, s + P < NS - P), False)
            return carry
        lax.fori_loop(0, UB, body, 0)

    x = jnp.broadcast_to(x_ref[...].astype(f32), (8, D))
    init_state()
    xn = _ln_bf16(x)
    wwait(wq_v, 0)
    qproj(xn, list(range(HKV)))
    pass1()
    x = mlp(attn_out(x))
    xn = _ln_bf16(x)
    qproj(xn, [HKV - 1])
    init_state()
    pass2a()
    qproj(xn, list(range(HKV - 1)))
    pass2b()
    x = mlp(attn_out(x))
    o_ref[...] = x[0:1, :].astype(o_ref.dtype)


@jax.jit
def pallas_interleave_layers__gqa_block_cached__dense_activation_mish__decode_kernel(
    A_x: jax.Array,
    A_k_cache: jax.Array,
    A_v_cache: jax.Array,
    A_wq: jax.Array,
    A_wo: jax.Array,
    B_x: jax.Array,
    B_w1: jax.Array,
    B_b1: jax.Array,
    B_w2: jax.Array,
):
    vm = pl.BlockSpec(memory_space=pltpu.VMEM)
    hb = pl.BlockSpec(memory_space=pl.ANY)
    out = pl.pallas_call(
        _kernel,
        out_shape=jax.ShapeDtypeStruct((1, D), bf16),
        in_specs=[vm, vm, hb, hb, hb, hb, hb, hb],
        out_specs=vm,
        scratch_shapes=[
            pltpu.VMEM((NSLOT, B, DH), bf16),
            pltpu.VMEM((NSLOT, B, DH), bf16),
            pltpu.VMEM((D, HQ * DH), bf16),
            pltpu.VMEM((HQ * DH, D), bf16),
            pltpu.VMEM((D, F), bf16),
            pltpu.VMEM((F, D), bf16),
            pltpu.VMEM((HKV, 8, DH), f32),
            pltpu.VMEM((HKV, 8, DH), f32),
            pltpu.VMEM((HKV, 8, DH), f32),
            pltpu.VMEM((HKV, 8, DH), f32),
            pltpu.VMEM((8, D), f32),
            pltpu.SMEM((HKV,), jnp.int32),
            pltpu.SemaphoreType.DMA((NSLOT,)),
            pltpu.SemaphoreType.DMA((NSLOT,)),
            pltpu.SemaphoreType.DMA((4,)),
        ],
        compiler_params=pltpu.CompilerParams(vmem_limit_bytes=128 * 1024 * 1024),
    )(A_x.reshape(1, D), B_b1, A_k_cache.reshape(T, B, DH), A_v_cache.reshape(T, B, DH),
      A_wq, A_wo, B_w1, B_w2)
    return out.reshape(1, 1, D)
```
